```python
import os as _os
_os.environ.setdefault("JAX_PLATFORMS", "cpu")
import jax
import jax.numpy as jnp

def _softmax(x, axis=-1):
    return jax.nn.softmax(x, axis=axis)
def _gelu(x):
    return jax.nn.gelu(x, approximate=True)
def _silu(x):
    return jax.nn.silu(x)
def _sigmoid(x):
    return jax.nn.sigmoid(x)
def _layernorm(x, axis=-1, eps=1e-5):
    m = jnp.mean(x, axis=axis, keepdims=True)
    v = jnp.var(x, axis=axis, keepdims=True)
    return (x - m) / jnp.sqrt(v + eps)
def _scatter_add(tgt, idx, src, axis=0):
    return tgt.at[idx].add(src)
def _segment_sum(src, seg, n):
    return jax.ops.segment_sum(src, seg, n)
class _Rng:
    def __init__(self, key):
        self._k = key
    def _next(self):
        self._k, sub = jax.random.split(self._k)
        return sub
    def normal(self, shape):
        return jax.random.normal(self._next(), shape, dtype=jnp.bfloat16)
    def randint(self, lo, hi, shape):
        return jax.random.randint(self._next(), shape, lo, hi, dtype=jnp.int32)
    def uniform(self, shape, lo=0.0, hi=1.0):
        return jax.random.uniform(self._next(), shape, jnp.bfloat16, lo, hi)
    def permutation(self, n):
        return jax.random.permutation(self._next(), n)


kernel_name = 'standalone__mha_softmax__near_ridge'

def setup_inputs():
    _rng = _Rng(jax.random.key(int.from_bytes(__import__("os").urandom(4), "little")))
    _w = (lambda a: (lambda t: t.astype(jnp.bfloat16) if jnp.issubdtype(t.dtype, jnp.floating) else t)(jnp.asarray(a)))
    B, H, Sq, Sk, D = 8, 16, 192, 1024, 256
    return {
        "q": _w((lambda *s: _rng.normal(s) * 0.4)(B, H, Sq, D)),
        "k": _w((lambda *s: _rng.normal(s) * 0.4)(B, H, Sk, D)),
        "v": _w((lambda *s: _rng.normal(s) * 0.05)(B, H, Sk, D)),
    }

def reference(q, k, v):
    scale = q.shape[-1] ** -0.5
    scores = jnp.einsum("bhqd,bhkd->bhqk", q, k) * scale
    p = _softmax(scores, axis=-1)
    return jnp.einsum("bhqk,bhkd->bhqd", p, v)
```

```python
import jax
import jax.numpy as jnp
from jax import lax
import jax.experimental.pallas as pl
import jax.experimental.pallas.tpu as pltpu

_LOG2E = 1.4426950408889634
_ROWS = 64
_LANES = 4
_AHEAD = 3
_WSTREAMS = 8
_WPER = 4


def _attend(q, k, v, scale):
    s = lax.dot_general(q, k, (((1,), (1,)), ((), ())), preferred_element_type=jnp.float32)
    m = jnp.max(s, axis=-1, keepdims=True)
    p = jnp.exp2((s - m) * (scale * _LOG2E))
    l = jnp.sum(p, axis=-1, keepdims=True)
    o = jnp.dot(p.astype(v.dtype), v, preferred_element_type=jnp.float32)
    return o * (1.0 / l)


@jax.jit
def pallas_standalone__mha_softmax__near_ridge_kernel(
    q: jax.Array,
    k: jax.Array,
    v: jax.Array,
):
    B, H, Sq, D = q.shape
    Sk = k.shape[2]
    nh = B * H
    qp, kp = Sq // _ROWS, Sk // _ROWS
    G, lead = _LANES, _AHEAD
    nb = lead + G
    per = nh * qp // _WSTREAMS
    scale = D ** -0.5

    part = kp // G
    pairs = [[("k", a, (G - 1 - a) * part + j), ("v", a, (G - 1 - a) * part + j)]
             for j in range(part) for a in range(G)]
    qpos = [(i + 1) * len(pairs) // qp - 1 for i in range(qp)]
    plan = []
    for i, pair in enumerate(pairs):
        plan += pair
        plan += [("q", 0, j) for j in range(qp) if qpos[j] == i]

    def kernel(q_hbm, k_hbm, v_hbm, o_hbm, qb, kb, vb, ob, sems, osem):
        def rem(x, n):
            return x % n if isinstance(x, int) else lax.rem(x, n)

        arrays = dict(q=(q_hbm, qb, qp), k=(k_hbm, kb, kp), v=(v_hbm, vb, kp))

        def issue(t, n):
            for kind, a, j in plan:
                h = t + a
                if isinstance(h, int) and not 0 <= h < nh:
                    continue
                slot = rem(h, nb)
                src, dst, pieces = arrays[kind]
                pltpu.make_async_copy(
                    src.at[h * pieces + j], dst.at[slot, j], sems.at[slot]
                ).start(priority=(n + 1) % 2)
                n += 1
            return n % 2

        def compute(h):
            slot = rem(h, nb)
            for ref in (qb, kb, vb):
                pltpu.make_async_copy(ref.at[slot], ref.at[slot], sems.at[slot]).wait()
            o = _attend(qb[slot].reshape(Sq, D), kb[slot].reshape(Sk, D),
                        vb[slot].reshape(Sk, D), scale)
            ob[h] = o.astype(ob.dtype).reshape(qp, _ROWS, D)

        def write(u0, u1, n):
            def body(u, _):
                for s in range(_WSTREAMS):
                    i = s * per + u
                    pltpu.make_async_copy(
                        ob.at[i // qp, rem(i, qp)], o_hbm.at[i], osem
                    ).start(priority=(s + 1 + n) % 2)
            lax.fori_loop(u0, u1, body, None)

        par = 0
        for t in range(-(G - 1), lead):
            par = issue(t, par)
        nfull = nh - (G - 1) - lead
        flip = len(plan) % 2

        def body(h, _):
            if flip:
                @pl.when(lax.rem(h, 2) == 0)
                def _():
                    issue(h + lead, par)

                @pl.when(lax.rem(h, 2) == 1)
                def _():
                    issue(h + lead, 1 - par)
            else:
                issue(h + lead, par)
            compute(h)

        lax.fori_loop(0, nfull, body, None)
        par2 = (par + flip * nfull) % 2
        par2 = issue(nfull + lead, par2)
        compute(nfull)
        for t in range(nfull + lead + 1, nh):
            par2 = issue(t, par2)
        h0 = nfull + 1

        def tail(h, _):
            compute(h)
            write((h - h0) * _WPER, (h - h0 + 1) * _WPER, par2)

        lax.fori_loop(h0, nh, tail, None)
        done = (nh - h0) * _WPER
        assert (_WSTREAMS - 1) * per + done <= h0 * qp
        write(done, per, par2)
        pltpu.make_async_copy(ob, ob, osem).wait()

    out = pl.pallas_call(
        kernel,
        out_shape=jax.ShapeDtypeStruct((nh * qp, _ROWS, D), q.dtype),
        in_specs=[pl.BlockSpec(memory_space=pl.ANY)] * 3,
        out_specs=pl.BlockSpec(memory_space=pl.ANY),
        scratch_shapes=[
            pltpu.VMEM((nb, qp, _ROWS, D), q.dtype),
            pltpu.VMEM((nb, kp, _ROWS, D), k.dtype),
            pltpu.VMEM((nb, kp, _ROWS, D), v.dtype),
            pltpu.VMEM((nh, qp, _ROWS, D), q.dtype),
            pltpu.SemaphoreType.DMA((nb,)),
            pltpu.SemaphoreType.DMA(()),
        ],
        compiler_params=pltpu.CompilerParams(
            vmem_limit_bytes=64 * 1024 * 1024, disable_bounds_checks=True),
    )(q.reshape(nh * qp, _ROWS, D), k.reshape(nh * kp, _ROWS, D), v.reshape(nh * kp, _ROWS, D))
    return out.reshape(B, H, Sq, D)
```

```python
import jax
import jax.numpy as jnp
from jax import lax
import jax.experimental.pallas as pl
import jax.experimental.pallas.tpu as pltpu

_LOG2E = 1.4426950408889634
_ROWS = 64
_LANES = 4
_LEAD = 6
_WSTREAMS = 8
_OVERLAP = 3


def _attend(q, k, v, scale):
    s = lax.dot_general(q, k, (((1,), (1,)), ((), ())),
                        preferred_element_type=jnp.float32)
    m = jnp.max(s, axis=-1, keepdims=True)
    p = jnp.exp2((s - m) * (scale * _LOG2E))
    l = jnp.sum(p, axis=-1, keepdims=True)
    o = jnp.dot(p.astype(v.dtype), v, preferred_element_type=jnp.float32)
    return o * (1.0 / l)


@jax.jit
def pallas_standalone__mha_softmax__near_ridge_kernel(
    q: jax.Array,
    k: jax.Array,
    v: jax.Array,
):
    B, H, Sq, D = q.shape
    Sk = k.shape[2]
    scale = D ** -0.5
    G = _LANES
    heads = B * H
    steps = heads // G
    qp, kp = Sq // _ROWS, Sk // _ROWS
    part = kp // G
    slots = pl.cdiv(_LEAD + G, G)
    wheads = heads // _WSTREAMS
    last = heads - 1 - _LEAD
    last_slot = (steps - 1) % slots
    assert Sq % _ROWS == 0 and Sk % (_ROWS * G) == 0 and qp <= G
    assert heads % _WSTREAMS == 0 and _WSTREAMS % G == 0
    assert 1 < _OVERLAP <= part and _LEAD >= G - 1 and last // G >= steps - wheads

    def kernel(q_hbm, k_hbm, v_hbm, o_hbm, q_buf, k_buf, v_buf, o_buf,
               sems, tail_sems, o_sem):
        def issue(t, final=False):
            s, b = t // G, t % G
            slot = s % slots

            def start(src, dst, sem, priority):
                pltpu.make_async_copy(src, dst, sem).start(priority=priority)

            for jj in range(part):
                if jj == 1:
                    @pl.when(b < qp)
                    def _():
                        for a in range(G):
                            start(q_hbm.at[(s + a * steps) * qp + b],
                                  q_buf.at[slot, a, b], sems.at[0, slot], (a + 1) % 2)
                j = b * part + jj
                if final and jj >= part - _OVERLAP:
                    k_sem, v_sem = tail_sems.at[0], tail_sems.at[1]
                else:
                    k_sem, v_sem = sems.at[1, slot], sems.at[2, slot]
                for a in range(G):
                    piece = (s + a * steps) * kp + j
                    start(k_hbm.at[piece], k_buf.at[slot, a, j], k_sem, 1)
                    start(v_hbm.at[piece], v_buf.at[slot, a, j], v_sem, 0)

        def wait_filled(buf, sem):
            pltpu.make_async_copy(buf, buf, sem).wait()

        def write(i):
            for j in range(qp):
                rows = pl.ds(pl.multiple_of(i * Sq + j * _ROWS, _ROWS), _ROWS)
                pltpu.make_async_copy(
                    o_buf.at[:, rows], o_hbm.at[:, rows], o_sem).start()

        def finished(s):
            return s - (steps - wheads)

        lax.fori_loop(0, _LEAD, lambda t, _: issue(t), None)

        def head(t, _):
            s, a = t // G, t % G
            slot = s % slots

            @pl.when(t < last)
            def _():
                issue(t + _LEAD)

            @pl.when(t == last)
            def _():
                issue(heads - 1, final=True)
                body, tail = pl.ds(0, kp - _OVERLAP), pl.ds(kp - _OVERLAP, _OVERLAP)
                wait_filled(q_buf.at[last_slot], sems.at[0, last_slot])
                wait_filled(k_buf.at[last_slot, :, body], sems.at[1, last_slot])
                wait_filled(v_buf.at[last_slot, :, body], sems.at[2, last_slot])
                lax.fori_loop(0, finished(last // G), lambda i, _: write(i), None)
                wait_filled(k_buf.at[last_slot, :, tail], tail_sems.at[0])
                wait_filled(v_buf.at[last_slot, :, tail], tail_sems.at[1])

            @pl.when(jnp.logical_and(a == 0, s < steps - 1))
            def _():
                wait_filled(q_buf.at[slot], sems.at[0, slot])
                wait_filled(k_buf.at[slot], sems.at[1, slot])
                wait_filled(v_buf.at[slot], sems.at[2, slot])

            o = _attend(q_buf[slot, a].reshape(Sq, D),
                        k_buf[slot, a].reshape(Sk, D),
                        v_buf[slot, a].reshape(Sk, D), scale)
            h = s + a * steps
            rows = pl.ds(pl.multiple_of((h % wheads) * Sq, Sq), Sq)
            o_buf[h // wheads, rows] = o.astype(o_buf.dtype)

            @pl.when(jnp.logical_and(t >= last, a == G - 1))
            def _():
                write(finished(s))

        lax.fori_loop(0, heads, head, None)
        pltpu.make_async_copy(o_buf, o_hbm, o_sem).wait()

    out = pl.pallas_call(
        kernel,
        out_shape=jax.ShapeDtypeStruct((_WSTREAMS, wheads * Sq, D), q.dtype),
        in_specs=[pl.BlockSpec(memory_space=pl.ANY)] * 3,
        out_specs=pl.BlockSpec(memory_space=pl.ANY),
        scratch_shapes=[
            pltpu.VMEM((slots, G, qp, _ROWS, D), q.dtype),
            pltpu.VMEM((slots, G, kp, _ROWS, D), k.dtype),
            pltpu.VMEM((slots, G, kp, _ROWS, D), v.dtype),
            pltpu.VMEM((_WSTREAMS, wheads * Sq, D), q.dtype),
            pltpu.SemaphoreType.DMA((3, slots)),
            pltpu.SemaphoreType.DMA((2,)),
            pltpu.SemaphoreType.DMA(()),
        ],
        compiler_params=pltpu.CompilerParams(
            vmem_limit_bytes=64 * 1024 * 1024,
            disable_bounds_checks=True,
            disable_semaphore_checks=True,
        ),
    )(q.reshape(heads * qp, _ROWS, D),
      k.reshape(heads * kp, _ROWS, D),
      v.reshape(heads * kp, _ROWS, D))
    return out.reshape(B, H, Sq, D)
```
